```python
import jax
import jax.numpy as jnp

def _softmax(x, axis=-1):
    return jax.nn.softmax(x, axis=axis)
def _gelu(x):
    return jax.nn.gelu(x, approximate=True)
def _silu(x):
    return jax.nn.silu(x)
def _sigmoid(x):
    return jax.nn.sigmoid(x)
def _layernorm(x, axis=-1, eps=1e-5):
    m = jnp.mean(x, axis=axis, keepdims=True)
    v = jnp.var(x, axis=axis, keepdims=True)
    return (x - m) / jnp.sqrt(v + eps)
def _scatter_add(tgt, idx, src, axis=0):
    return tgt.at[idx].add(src)
def _segment_sum(src, seg, n):
    return jax.ops.segment_sum(src, seg, n)
class _Rng:
    def __init__(self, key):
        self._k = key
    def _next(self):
        self._k, sub = jax.random.split(self._k)
        return sub
    def normal(self, shape):
        return jax.random.normal(self._next(), shape, dtype=jnp.bfloat16)
    def randint(self, lo, hi, shape):
        return jax.random.randint(self._next(), shape, lo, hi, dtype=jnp.int32)
    def uniform(self, shape, lo=0.0, hi=1.0):
        return jax.random.uniform(self._next(), shape, jnp.bfloat16, lo, hi)
    def permutation(self, n):
        return jax.random.permutation(self._next(), n)


kernel_name = 'standalone__batchnorm__prompt'

def setup_inputs():
    _rng = _Rng(jax.random.key(int.from_bytes(__import__("os").urandom(4), "little")))
    _w = (lambda a: (lambda t: t.astype(jnp.bfloat16) if jnp.issubdtype(t.dtype, jnp.floating) else t)(jnp.asarray(a)))
    B, S, C = 2, 2048, 1024
    K = 3
    return {
        "x": _w((lambda *s: _rng.normal(s) * 0.05)(B, S, C)),
        "w": _w((lambda *s: _rng.normal(s) * 0.05)(K, C, C) * (1.0 / (K * C) ** 0.5)),
        "mean": _w((lambda *s: _rng.normal(s) * 0.05)(C) * 0.1),
        "var": _w(jnp.abs((lambda *s: _rng.normal(s) * 0.05)(C)) + 0.5),
        "g": _w((lambda *s: _rng.normal(s) * 0.05)(C) + 1.0),
        "b": _w((lambda *s: _rng.normal(s) * 0.05)(C) * 0.1),
    }

def reference(x, w, mean, var, g, b):
    K = 3
    P = K // 2
    S = x.shape[1]
    xp = jnp.pad(x, ((0, 0), (P, P), (0, 0)))
    y = sum(jnp.einsum('bsc,cd->bsd', xp[:, k:k + S, :], w[k]) for k in range(K))
    inv_std = 1.0 / jnp.sqrt(var + 1e-5)
    y = (y - mean) * (g * inv_std) + b
    return _silu(y)
```

```python
import jax, jax.numpy as jnp
import numpy as np
import jax.experimental.pallas as pl
import jax.experimental.pallas.tpu as pltpu

F32 = jnp.float32
BF = jnp.bfloat16
U32 = jnp.uint32
A_ = 2.0 / 3.0
B_ = 1.5
NA = 2 * A_**2 * (A_**2 - B_**2)
NB = 2 * B_**2 * (B_**2 - A_**2)
CC = A_**2 + B_**2

def up(u, i):
    return pltpu.unpack_elementwise(u, index=i, packed_dtype=BF, unpacked_dtype=F32)
def pk(a, b):
    return pltpu.pack_elementwise([a, b], packed_dtype=BF)

def wino_in(d0, d1, d2, d3, d4, d5):
    pa = d4 - (B_**2) * d2; qa = A_ * d3 - B_ * d1
    pb = d4 - (A_**2) * d2; qb = B_ * d3 - A_ * d1
    return [d0 - CC * d2 + d4, pa + qa, pa - qa, pb + qb, pb - qb, d1 - CC * d3 + d5]

def make(R=512, tn=256, vmem=100, act='tanh', xn0=3, nm_run=None, TC=16, RC=16, order='post', fine=1):
    B, S, C = 2, 2048, 1024
    NCB = C // 128
    CPB = S // R
    NM = B * CPB
    NMR = nm_run or NM
    NN = C // tn
    TT = R // 4
    PAD = 16
    CBN = tn // 128
    def kernel(x_hbm, w_hbm, mean_ref, var_ref, g_ref, b_ref, o_hbm, xs, wst, os_, scsh, xsem, wsem, osem, *GT):
        G = GT[:NN]; T = GT[NN:]
        def x_copies(m):
            b, c = divmod(m, CPB)
            lo = 0 if c == 0 else c * R + PAD
            hi = S if c == CPB - 1 else (c + 1) * R + PAD
            return [pltpu.make_async_copy(x_hbm.at[b, pl.ds(lo, hi - lo), pl.ds(cb * 128, 128)],
                                          xs.at[b, cb, pl.ds(PAD + lo, hi - lo), :], xsem.at[m]) for cb in range(NCB)]
        def w_copies(n):
            return [pltpu.make_async_copy(w_hbm.at[k, :, pl.ds(cb * 128, 128)], wst.at[k, cb], wsem.at[n])
                    for k in range(3) for cb in range(n * CBN, (n + 1) * CBN)]
        def o_copies(m, n):
            b, c = divmod(m, CPB)
            return [pltpu.make_async_copy(os_.at[b, cb, pl.ds(c * R, R), :], o_hbm.at[b, pl.ds(c * R, R), pl.ds(cb * 128, 128)], osem.at[0])
                    for cb in range(n * CBN, (n + 1) * CBN)]
        for cp in w_copies(0): cp.start()
        for cp in x_copies(0): cp.start()
        z = jnp.zeros((PAD, 128), BF)
        for b in range(B):
            for cb in range(NCB):
                xs[b, cb, 0:PAD, :] = z
                xs[b, cb, PAD + S:PAD + S + PAD, :] = z
        f = lambda r: r[...].astype(F32).reshape(1, C)
        sc = f(g_ref) * jax.lax.rsqrt(f(var_ref) + 1e-5)
        sh = f(b_ref) - f(mean_ref) * sc
        if act == 'tanh':
            sc = sc * 0.5; sh = sh * 0.5
        scsh[0:1, :] = sc
        scsh[1:2, :] = sh

        def g_transform(n, i, r0, r1):
            cb = n * CBN + i
            wu = [wst.at[k, cb].bitcast(U32) for k in range(3)]
            cs = slice(i * 128, (i + 1) * 128)
            for r in range(r0, r1, RC):
                hs = slice(r, r + RC)
                u0, u1, u2 = wu[0][hs, :], wu[1][hs, :], wu[2][hs, :]
                G[n][0, hs, cs] = u0
                G[n][5, hs, cs] = u2
                res = []
                for h in range(2):
                    w0, w1, w2 = up(u0, h), up(u1, h), up(u2, h)
                    ea = w0 * (1 / NA) + w2 * (A_**2 / NA); oa = w1 * (A_ / NA)
                    eb = w0 * (1 / NB) + w2 * (B_**2 / NB); ob = w1 * (B_ / NB)
                    res.append([ea + oa, ea - oa, eb + ob, eb - ob])
                for j in range(4):
                    G[n][1 + j, hs, cs] = pk(res[0][j], res[1][j])

        def t_transform(m, cb, t_lo, t_hi):
            b, c = divmod(m, CPB)
            xu = xs.at[b, cb].bitcast(U32)
            base = PAD // 2 + c * (R // 2)
            H = TC // 2
            for t0_ in range(t_lo, t_hi, TC):
                rb = base + 2 * t0_
                u = [xu[pl.ds(rb + o, H, stride=4), :] for o in range(-1, 5)]
                lo = [up(v, 0) for v in u]; hi = [up(v, 1) for v in u]
                ta = wino_in(hi[0], lo[1], hi[1], lo[2], hi[2], lo[3])
                tb = wino_in(hi[2], lo[3], hi[3], lo[4], hi[4], lo[5])
                for j in range(6):
                    T[m % 2][j, t0_ // 2:(t0_ + TC) // 2, cb * 128:(cb + 1) * 128] = pk(ta[j], tb[j])

        def step(m, n):
            b, c = divmod(m, CPB)
            cs = slice(n * tn, (n + 1) * tn)
            mm = [jnp.dot(pltpu.bitcast(T[m % 2][j], BF), pltpu.bitcast(G[n][j], BF), preferred_element_type=F32) for j in range(6)]
            s12 = mm[1] + mm[2]; d12 = mm[1] - mm[2]; s34 = mm[3] + mm[4]; d34 = mm[3] - mm[4]
            y0 = mm[0] + s12 + s34
            y1 = A_ * d12 + B_ * d34
            y2 = (A_**2) * s12 + (B_**2) * s34
            y3 = (A_**3) * d12 + (B_**3) * d34 + mm[5]
            sc = scsh[0:1, cs]; sh = scsh[1:2, cs]
            def a_(y):
                y = y * sc + sh
                if act == 'tanh':
                    return y * jnp.tanh(y) + y
                return y * jax.nn.sigmoid(y)
            p01 = pk(a_(y0), a_(y1))
            p23 = pk(a_(y2), a_(y3))
            for i in range(CBN):
                cb = n * CBN + i
                ou = os_.at[b, cb].bitcast(U32)
                ou[pl.ds(c * (R // 2), TT, stride=2), :] = p01[:, i * 128:(i + 1) * 128]
                ou[pl.ds(c * (R // 2) + 1, TT, stride=2), :] = p23[:, i * 128:(i + 1) * 128]

        for cp in w_copies(0): cp.wait()
        if NN > 1:
            for cp in w_copies(1): cp.start()
        for i in range(CBN): g_transform(0, i, 0, C // 2)
        for cp in x_copies(0): cp.wait()
        if NN > 2:
            for cp in w_copies(2): cp.start()
        else:
            for cp in x_copies(1): cp.start()
        for cb in range(NCB): t_transform(0, cb, 0, TT)
        for m in range(NMR):
            for n in range(NN):
                def prep():
                    if m == 0 and n + 1 < NN:
                        for cp in w_copies(n + 1): cp.wait()
                        if n + 3 < NN:
                            for cp in w_copies(n + 3): cp.start()
                        elif n + 3 == NN:
                            for cp in x_copies(1): cp.start()
                        for i in range(CBN): g_transform(n + 1, i, 0, C // 2)
                    tn0 = xn0 if m == 0 else 0
                    if m + 1 < NMR and n >= tn0:
                        if n == tn0:
                            for cp in x_copies(m + 1): cp.wait()
                            if m + 2 < NMR:
                                for cp in x_copies(m + 2): cp.start()
                        nn = NN - tn0
                        for cb in range((n - tn0) * NCB // nn, (n - tn0 + 1) * NCB // nn):
                            t_transform(m + 1, cb, 0, TT)
                if order == 'pre':
                    prep()
                step(m, n)
                for cp in o_copies(m, n): cp.start()
                if order == 'post':
                    prep()
        if NMR == 1:
            for cp in x_copies(1): cp.wait()
        for m in range(NMR):
            for n in range(NN):
                for cp in o_copies(m, n): cp.wait()

    def fn(x, w, mean, var, g, b):
        vspec = pl.BlockSpec((C,), lambda: (0,))
        return pl.pallas_call(
            kernel,
            in_specs=[pl.BlockSpec(memory_space=pl.ANY)] * 2 + [vspec] * 4,
            out_specs=pl.BlockSpec(memory_space=pl.ANY),
            out_shape=jax.ShapeDtypeStruct((B, S, C), x.dtype),
            scratch_shapes=[
                pltpu.VMEM((B, NCB, S + 2 * PAD, 128), BF),
                pltpu.VMEM((3, NCB, C, 128), BF),
                pltpu.VMEM((B, NCB, S, 128), BF),
                pltpu.VMEM((8, C), F32),
                pltpu.SemaphoreType.DMA((NM,)),
                pltpu.SemaphoreType.DMA((NN,)),
                pltpu.SemaphoreType.DMA((1,)),
            ] + [pltpu.VMEM((6, C // 2, tn), U32) for _ in range(NN)] + [pltpu.VMEM((6, TT // 2, C), U32) for _ in range(2)],
            compiler_params=pltpu.CompilerParams(vmem_limit_bytes=vmem * 2**20),
        )(x, w, mean, var, g, b)
    return fn


_fn = make()


@jax.jit
def pallas_standalone__batchnorm__prompt_kernel(x, w, mean, var, g, b):
    return _fn(x, w, mean, var, g, b)
```

```python
import functools as ft
import jax, jax.numpy as jnp
import numpy as np
import jax.experimental.pallas as pl
import jax.experimental.pallas.tpu as pltpu

F32 = jnp.float32
BF = jnp.bfloat16
U32 = jnp.uint32
A_ = 2.0 / 3.0
B_ = 1.5
NA = 2 * A_**2 * (A_**2 - B_**2)
NB = 2 * B_**2 * (B_**2 - A_**2) * A_**2
CC = A_**2 + B_**2

def up(u, i):
    return pltpu.unpack_elementwise(u, index=i, packed_dtype=BF, unpacked_dtype=F32)
def pk(a, b):
    return pltpu.pack_elementwise([a, b], packed_dtype=BF)

def wino_in(d0, d1, d2, d3, d4, d5):
    a1 = A_ * d1
    pa = (A_**2) * d4 - d2; qa = (A_**3) * d3 - a1
    pb = d4 - (A_**2) * d2; qb = B_ * d3 - a1
    return [d0 - CC * d2 + d4, pa + qa, pa - qa, pb + qb, pb - qb, d1 - CC * d3 + d5]
SA = 1.0 / (NA * A_**2)
SB = 1.0 / NB

def make(R=512, vmem=100, act='tanh', nm_run=None, pin=True, pinpos=(56, 896), sched='rowfirst', flags=None, wpos=3, first_order='xw', mode='peel01'):
    B, S, C = 2, 2048, 1024
    NCB = C // 128
    CPB = S // R
    NM = B * CPB
    NMR = nm_run or NM
    NN = NCB
    TT = R // 4
    HT = TT // 2
    PAD = 16
    TC = 16
    def kernel(x_hbm, w_hbm, mean_ref, var_ref, g_ref, b_ref, o_hbm, xs, wst, os_, scsh, xsem, wsem, osem, *GT):
        G = GT[:NN]; T = GT[NN:]
        def bc(m):
            if isinstance(m, int):
                return divmod(m, CPB)
            return m // CPB, m % CPB
        def rowoff(c):
            return c * R if isinstance(c, int) else pl.multiple_of(c * R, R)
        def x_copies(m):
            b, c = bc(m)
            lo = 0 if c == 0 else c * R + PAD
            hi = S if c == CPB - 1 else (c + 1) * R + PAD
            return [pltpu.make_async_copy(x_hbm.at[b, pl.ds(lo, hi - lo), pl.ds(cb * 128, 128)],
                                          xs.at[b, cb, pl.ds(PAD + lo, hi - lo), :], xsem.at[m]) for cb in range(NCB)]
        def w_copies(n):
            return [pltpu.make_async_copy(w_hbm.at[k, :, pl.ds(n * 128, 128)], wst.at[k, n], wsem.at[n]) for k in range(3)]
        def o_copies(m, n):
            b, c = bc(m)
            lo = rowoff(c)
            return [pltpu.make_async_copy(os_.at[b, n, pl.ds(lo, R), :], o_hbm.at[b, pl.ds(lo, R), pl.ds(n * 128, 128)], osem.at[0])]
        def start(cps):
            for cp in cps: cp.start()
        def wait(cps):
            for cp in cps: cp.wait()
        if first_order == 'xw':
            start(x_copies(0)); start(w_copies(0))
        else:
            start(w_copies(0)); start(x_copies(0))
        start(w_copies(1))
        z = jnp.zeros((PAD, 128), BF)
        for b in range(B):
            for cb in range(NCB):
                xs[b, cb, 0:PAD, :] = z
                xs[b, cb, PAD + S:PAD + S + PAD, :] = z
        f = lambda r: r[...].astype(F32).reshape(1, C)
        sc = f(g_ref) * jax.lax.rsqrt(f(var_ref) + 1e-5)
        sh = f(b_ref) - f(mean_ref) * sc
        if act == 'tanh':
            sc = sc * 0.5; sh = sh * 0.5
        scsh[0:1, :] = sc
        scsh[1:2, :] = sh
        zero = (pltpu.bitcast(jnp.broadcast_to(sc[:, 0:128], (8, 128)), U32) >> 16) >> 16

        def g_piece(n, r):
            wu = [wst.at[k, n].bitcast(U32) for k in range(3)]
            hs = slice(r, r + 8)
            u0, u1, u2 = wu[0][hs, :], wu[1][hs, :], wu[2][hs, :]
            res = []
            for h in range(2):
                w0, w1, w2 = up(u0, h), up(u1, h), up(u2, h)
                o = A_ * w1
                ea = w0 + (A_**2) * w2
                eb = (A_**2) * w0 + w2
                res.append([ea + o, ea - o, eb + o, eb - o])
            acc = None
            for j in range(4):
                p = pk(res[0][j], res[1][j])
                G[n][j, hs, :] = p
                acc = p if acc is None else acc | p
            return acc

        def t_piece(m, slot, cb, t0_):
            b, c = bc(m)
            xu = xs.at[b, cb, pl.ds(rowoff(c), R + 2 * PAD), :].bitcast(U32)
            rb = PAD // 2 + 2 * t0_
            u = [xu[pl.ds(rb + o, 8, stride=4), :] for o in range(-1, 5)]
            lo = [up(v, 0) for v in u[1:]]; hi = [up(v, 1) for v in u[:5]]
            lo = [None] + lo
            ta = wino_in(hi[0], lo[1], hi[1], lo[2], hi[2], lo[3])
            tb = wino_in(hi[2], lo[3], hi[3], lo[4], hi[4], lo[5])
            acc = None
            for j in range(6):
                p = pk(ta[j], tb[j])
                T[slot][j, t0_ // 2:t0_ // 2 + 8, cb * 128:(cb + 1) * 128] = p
                acc = p if acc is None else acc | p
            return acc

        def step(m, slot, n, fillers, hooks=()):
            b, c = bc(m)
            cs = slice(n * 128, (n + 1) * 128)
            mm = []
            nf = len(fillers)
            for j in range(6):
                for (hp, hf) in hooks:
                    if hp == j: hf()
                zz = None
                for fl in fillers[j * nf // 6:(j + 1) * nf // 6]:
                    a = fl()
                    zz = a if zz is None else zz | a
                tref = T[slot]
                if zz is not None and pin:
                    zz = zz & zero
                    pr, pc = pinpos
                    rowblk = jnp.concatenate(
                        ([tref[j, pr:pr + 8, 0:pc]] if pc > 0 else []) + [tref[j, pr:pr + 8, pc:pc + 128] | zz] + ([tref[j, pr:pr + 8, pc + 128:]] if pc + 128 < C else []), axis=1)
                    lhs = jnp.concatenate(([tref[j, 0:pr, :]] if pr > 0 else []) + [rowblk] + ([tref[j, pr + 8:, :]] if pr + 8 < HT else []), axis=0)
                else:
                    lhs = tref[j]
                if j == 0:
                    rhs = wst.at[0, n].bitcast(U32)[...]
                elif j == 5:
                    rhs = wst.at[2, n].bitcast(U32)[...]
                else:
                    rhs = G[n][j - 1]
                mm.append(jnp.dot(pltpu.bitcast(lhs, BF), pltpu.bitcast(rhs, BF), preferred_element_type=F32))
            s12 = mm[1] + mm[2]; d12 = mm[1] - mm[2]; s34 = mm[3] + mm[4]; d34 = mm[3] - mm[4]
            y0 = mm[0] + SA * s12 + SB * s34
            y1 = (SA * A_) * d12 + (SB * B_) * d34
            y2 = (SA * A_**2) * s12 + (SB * B_**2) * s34
            y3 = (SA * A_**3) * d12 + (SB * B_**3) * d34 + mm[5]
            sc = scsh[0:1, cs]; sh = scsh[1:2, cs]
            def a_(y):
                y = y * sc + sh
                if act == 'tanh':
                    return y * jnp.tanh(y) + y
                return y * jax.nn.sigmoid(y)
            ou = os_.at[b, n, pl.ds(rowoff(c), R), :].bitcast(U32)
            ou[pl.ds(0, TT, stride=2), :] = pk(a_(y0), a_(y1))
            ou[pl.ds(1, TT, stride=2), :] = pk(a_(y2), a_(y3))
            start(o_copies(m, n))

        def tfill(m, slot=None):
            slot = m % 2 if slot is None else slot
            return [ft.partial(t_piece, m, slot, cb, t) for cb in range(NCB) for t in range(0, TT, TC)]
        def gfill(n):
            return [ft.partial(g_piece, n, r) for r in range(0, C // 2, 8)]
        def part(lst, i, k):
            return lst[i * len(lst) // k:(i + 1) * len(lst) // k]

        if first_order == 'xw':
            wait(x_copies(0)); start(w_copies(2))
            for fl in tfill(0): fl()
            wait(w_copies(0)); start(w_copies(3))
            for fl in gfill(0): fl()
        else:
            wait(w_copies(0)); start(w_copies(2))
            for fl in gfill(0): fl()
            wait(x_copies(0)); start(w_copies(3))
            for fl in tfill(0): fl()
        wait(w_copies(1))
        for n in range(NN):
            fl = []
            hooks = []
            if n + 1 < NN:
                fl += gfill(n + 1)
            if n + 2 < NN:
                def hk(n=n):
                    wait(w_copies(n + 2))
                    if n + 4 < NN: start(w_copies(n + 4))
                    elif n + 4 == NN: start(x_copies(1))
                    elif n + 4 == NN + 1: start(x_copies(2))
                hooks.append((wpos, hk))
            elif n + 2 == NN:
                def hk(n=n):
                    wait(x_copies(1))
                    for m_ in range(3, 6): start(x_copies(m_))
                hooks.append((wpos, hk))
            if n >= NN - 2:
                if n == NN - 1:
                    fl += tfill(1)
            step(0, 0, n, fl, hooks)
        def chunk(m, slot, last=False):
            if isinstance(m, int):
                tf = [] if m + 1 >= NM else tfill(m + 1, 1 - slot)
            else:
                tf = tfill(jnp.minimum(m + 1, NM - 1), 1 - slot)
            for n in range(NN):
                step(m, slot, n, part(tf, n, NN))
        if mode == 'peel01':
            wait(x_copies(2))
            for m_ in range(6, NM): start(x_copies(m_))
            chunk(1, 1)
            for m_ in range(3, NM): wait(x_copies(m_))
            def body(i, carry):
                m = 2 * i + 2
                chunk(m, 0)
                chunk(m + 1, 1)
                return carry
            jax.lax.fori_loop(0, (NM - 2) // 2, body, 0)
        elif mode == 'pred':
            def body(i, carry):
                m = 2 * i + 1
                @pl.when(i == 0)
                def _():
                    wait(x_copies(2))
                    for m_ in range(6, NM): start(x_copies(m_))
                @pl.when(i == 1)
                def _():
                    for m_ in range(3, NM): wait(x_copies(m_))
                chunk(m, 1)
                @pl.when(m + 1 < NM)
                def _():
                    chunk(m + 1, 0)
                return carry
            jax.lax.fori_loop(0, NM // 2, body, 0)
        elif mode == 'peel07':
            def body(i, carry):
                m = 2 * i + 1
                @pl.when(i == 0)
                def _():
                    wait(x_copies(2))
                    for m_ in range(6, NM): start(x_copies(m_))
                @pl.when(i == 1)
                def _():
                    for m_ in range(3, NM): wait(x_copies(m_))
                chunk(m, 1)
                chunk(m + 1, 0)
                return carry
            jax.lax.fori_loop(0, (NM - 2) // 2, body, 0)
            chunk(NM - 1, 1)
        else:
            for m in range(1, NM):
                if m == 1:
                    wait(x_copies(2))
                    for m_ in range(6, NM): start(x_copies(m_))
                if m == 2:
                    for m_ in range(3, NM): wait(x_copies(m_))
                chunk(m, m % 2)
        for m in range(NM):
            for n in range(NN):
                wait(o_copies(m, n))

    def fn(x, w, mean, var, g, b):
        vspec = pl.BlockSpec((C,), lambda: (0,))
        return pl.pallas_call(
            kernel,
            in_specs=[pl.BlockSpec(memory_space=pl.ANY)] * 2 + [vspec] * 4,
            out_specs=pl.BlockSpec(memory_space=pl.ANY),
            out_shape=jax.ShapeDtypeStruct((B, S, C), x.dtype),
            scratch_shapes=[
                pltpu.VMEM((B, NCB, S + 2 * PAD, 128), BF),
                pltpu.VMEM((3, NCB, C, 128), BF),
                pltpu.VMEM((B, NCB, S, 128), BF),
                pltpu.VMEM((8, C), F32),
                pltpu.SemaphoreType.DMA((NM,)),
                pltpu.SemaphoreType.DMA((NN,)),
                pltpu.SemaphoreType.DMA((1,)),
            ] + [pltpu.VMEM((4, C // 2, 128), U32) for _ in range(NN)] + [pltpu.VMEM((6, HT, C), U32) for _ in range(2)],
            compiler_params=pltpu.CompilerParams(vmem_limit_bytes=vmem * 2**20, flags=flags),
        )(x, w, mean, var, g, b)
    return fn


_fn = make()


@jax.jit
def pallas_standalone__batchnorm__prompt_kernel(x, w, mean, var, g, b):
    return _fn(x, w, mean, var, g, b)
```

```python
import functools as ft
import jax, jax.numpy as jnp
import numpy as np
import jax.experimental.pallas as pl
import jax.experimental.pallas.tpu as pltpu

F32 = jnp.float32
BF = jnp.bfloat16
U32 = jnp.uint32
A_ = 2.0 / 3.0
B_ = 1.5
NA = 2 * A_**2 * (A_**2 - B_**2)
NB = 2 * B_**2 * (B_**2 - A_**2) * A_**2
CC = A_**2 + B_**2

def up(u, i):
    return pltpu.unpack_elementwise(u, index=i, packed_dtype=BF, unpacked_dtype=F32)
def pk(a, b):
    return pltpu.pack_elementwise([a, b], packed_dtype=BF)

def wino_in(d0, d1, d2, d3, d4, d5):
    a1 = A_ * d1
    pa = (A_**2) * d4 - d2; qa = (A_**3) * d3 - a1
    pb = d4 - (A_**2) * d2; qb = B_ * d3 - a1
    return [d0 - CC * d2 + d4, pa + qa, pa - qa, pb + qb, pb - qb, d1 - CC * d3 + d5]
SA = 1.0 / (NA * A_**2)
SB = 1.0 / NB

def make(R=512, vmem=100, act='tanh', nm_run=None, pin=True, pinpos=(56, 896), sched='rowfirst', flags=None, wpos=3, first_order='xw', JORD=(0, 5, 1, 2, 3, 4), hpos=0, h0pos=3, ahead=3, gspill=2):
    B, S, C = 2, 2048, 1024
    NCB = C // 128
    CPB = S // R
    NM = B * CPB
    NMR = nm_run or NM
    NN = NCB
    TT = R // 4
    HT = TT // 2
    PAD = 16
    TC = 16
    def kernel(x_hbm, w_hbm, mean_hbm, var_hbm, g_hbm, b_hbm, o_hbm, xs, wst, os_, scsh, v0, v1, v2, v3, xsem, wsem, osem, vsem, *GT):
        vecs = (v0, v1, v2, v3)
        G = GT[:NN]; T = GT[NN:]
        def bc(m):
            if isinstance(m, int):
                return divmod(m, CPB)
            return m // CPB, m % CPB
        def rowoff(c):
            return c * R if isinstance(c, int) else pl.multiple_of(c * R, R)
        def x_copies(m):
            b, c = bc(m)
            lo = 0 if c == 0 else c * R + PAD
            hi = S if c == CPB - 1 else (c + 1) * R + PAD
            return [pltpu.make_async_copy(x_hbm.at[b, pl.ds(lo, hi - lo), pl.ds(cb * 128, 128)],
                                          xs.at[b, cb, pl.ds(PAD + lo, hi - lo), :], xsem.at[m]) for cb in range(NCB)]
        def w_copies(n):
            return [pltpu.make_async_copy(w_hbm.at[k, :, pl.ds(n * 128, 128)], wst.at[k, n], wsem.at[n]) for k in range(3)]
        def o_copies(m, n):
            b, c = bc(m)
            lo = rowoff(c)
            return [pltpu.make_async_copy(os_.at[b, n, pl.ds(lo, R), :], o_hbm.at[b, pl.ds(lo, R), pl.ds(n * 128, 128)], osem.at[0])]
        def start(cps):
            for cp in cps: cp.start()
        def wait(cps):
            for cp in cps: cp.wait()
        v_copies = [pltpu.make_async_copy(src, vecs[i], vsem.at[0]) for i, src in enumerate((mean_hbm, var_hbm, g_hbm, b_hbm))]
        start(v_copies)
        start(x_copies(0)); start(w_copies(0))
        z = jnp.zeros((PAD, 128), BF)
        for b in range(B):
            for cb in range(NCB):
                xs[b, cb, 0:PAD, :] = z
                xs[b, cb, PAD + S:PAD + S + PAD, :] = z
        def bn_params():
            f = lambda i: vecs[i][...].astype(F32).reshape(1, C)
            sc = f(2) * jax.lax.rsqrt(f(1) + 1e-5)
            sh = f(3) - f(0) * sc
            if act == 'tanh':
                sc = sc * 0.5; sh = sh * 0.5
            scsh[0:1, :] = sc
            scsh[1:2, :] = sh
            return (pltpu.bitcast(jnp.broadcast_to(sc[:, 0:128], (8, 128)), U32) >> 16) >> 16
        zero_box = []

        def g_piece(n, r):
            wu = [wst.at[k, n].bitcast(U32) for k in range(3)]
            hs = slice(r, r + 8)
            u0, u1, u2 = wu[0][hs, :], wu[1][hs, :], wu[2][hs, :]
            res = []
            for h in range(2):
                w0, w1, w2 = up(u0, h), up(u1, h), up(u2, h)
                o = A_ * w1
                ea = w0 + (A_**2) * w2
                eb = (A_**2) * w0 + w2
                res.append([ea + o, ea - o, eb + o, eb - o])
            acc = None
            for j in range(4):
                p = pk(res[0][j], res[1][j])
                G[n][j, hs, :] = p
                acc = p if acc is None else acc | p
            return acc

        def t_piece(m, slot, cb, t0_):
            b, c = bc(m)
            xu = xs.at[b, cb, pl.ds(rowoff(c), R + 2 * PAD), :].bitcast(U32)
            rb = PAD // 2 + 2 * t0_
            u = [xu[pl.ds(rb + o, 8, stride=4), :] for o in range(-1, 5)]
            lo = [up(v, 0) for v in u[1:]]; hi = [up(v, 1) for v in u[:5]]
            lo = [None] + lo
            ta = wino_in(hi[0], lo[1], hi[1], lo[2], hi[2], lo[3])
            tb = wino_in(hi[2], lo[3], hi[3], lo[4], hi[4], lo[5])
            acc = None
            for j in range(6):
                p = pk(ta[j], tb[j])
                T[slot][j, t0_ // 2:t0_ // 2 + 8, cb * 128:(cb + 1) * 128] = p
                acc = p if acc is None else acc | p
            return acc

        def step(m, slot, n, fmap, hooks=()):
            b, c = bc(m)
            cs = slice(n * 128, (n + 1) * 128)
            mm = {}
            for pos, j in enumerate(JORD):
                for (hp, hf) in hooks:
                    if hp == pos: hf()
                zz = None
                for fl in fmap.get(pos, []):
                    a = fl()
                    zz = a if zz is None else zz | a
                tref = T[slot]
                if zz is not None and pin:
                    zz = zz & zero_box[0]
                    pr, pc = pinpos
                    rowblk = jnp.concatenate(
                        ([tref[j, pr:pr + 8, 0:pc]] if pc > 0 else []) + [tref[j, pr:pr + 8, pc:pc + 128] | zz] + ([tref[j, pr:pr + 8, pc + 128:]] if pc + 128 < C else []), axis=1)
                    lhs = jnp.concatenate(([tref[j, 0:pr, :]] if pr > 0 else []) + [rowblk] + ([tref[j, pr + 8:, :]] if pr + 8 < HT else []), axis=0)
                else:
                    lhs = tref[j]
                if j == 0:
                    rhs = wst.at[0, n].bitcast(U32)[...]
                elif j == 5:
                    rhs = wst.at[2, n].bitcast(U32)[...]
                else:
                    rhs = G[n][j - 1]
                mm[j] = jnp.dot(pltpu.bitcast(lhs, BF), pltpu.bitcast(rhs, BF), preferred_element_type=F32)
            s12 = mm[1] + mm[2]; d12 = mm[1] - mm[2]; s34 = mm[3] + mm[4]; d34 = mm[3] - mm[4]
            y0 = mm[0] + SA * s12 + SB * s34
            y1 = (SA * A_) * d12 + (SB * B_) * d34
            y2 = (SA * A_**2) * s12 + (SB * B_**2) * s34
            y3 = (SA * A_**3) * d12 + (SB * B_**3) * d34 + mm[5]
            sc = scsh[0:1, cs]; sh = scsh[1:2, cs]
            def a_(y):
                y = y * sc + sh
                if act == 'tanh':
                    return y * jnp.tanh(y) + y
                return y * jax.nn.sigmoid(y)
            ou = os_.at[b, n, pl.ds(rowoff(c), R), :].bitcast(U32)
            ou[pl.ds(0, TT, stride=2), :] = pk(a_(y0), a_(y1))
            ou[pl.ds(1, TT, stride=2), :] = pk(a_(y2), a_(y3))
            start(o_copies(m, n))

        def tfill(m, slot=None):
            slot = m % 2 if slot is None else slot
            return [ft.partial(t_piece, m, slot, cb, t) for cb in range(NCB) for t in range(0, TT, TC)]
        def gfill(n):
            return [ft.partial(g_piece, n, r) for r in range(0, C // 2, 8)]
        def part(lst, i, k):
            return lst[i * len(lst) // k:(i + 1) * len(lst) // k]

        Q = [('x', 0), ('w', 0), ('x', 1)] + [('w', n) for n in range(1, NN)] + [('x', m) for m in range(2, NM)]
        cps = lambda it: x_copies(it[1]) if it[0] == 'x' else w_copies(it[1])
        qpos = [2]
        def issue(k=1):
            for _ in range(k):
                if qpos[0] < len(Q):
                    start(cps(Q[qpos[0]])); qpos[0] += 1
        def arrive(*items):
            issue(max(Q.index(it) for it in items) + 1 - qpos[0])
            with jax.named_scope('wait_' + ''.join(f'{a}{b}' for a, b in items)):
                for it in items: wait(cps(it))
            last = max(Q.index(it) for it in items)
            issue(last + 1 + ahead - qpos[0])
        arrive(('x', 0))
        for fl in tfill(0, 2): fl()
        wait(v_copies)
        zero_box.append(bn_params())
        arrive(('w', 0))
        g0 = gfill(0)
        step(0, 2, 0, {0: part(g0, 0, 2), 1: part(g0, 1, 2)})
        arrive(('x', 1))
        for fl in tfill(1, 1): fl()
        waits = {0: [('w', 1)], 1: [('w', 2)], 2: [('w', 3)], 3: [('w', 4), ('w', 5)], 5: [('w', 6), ('w', 7), ('x', 2)]}
        for n in range(NN):
            fm, hooks, carry = {}, [], {}
            need = waits.get(n, [])
            k0 = 0
            if need:
                k0 = h0pos if n == 0 else hpos
                hooks.append((k0, lambda need=need: arrive(*need)))
            if n + 1 < NN:
                gl = gfill(n + 1)
                nd = (6 - k0) + gspill
                fm = {k: part(gl, k - k0, nd) for k in range(k0, 6)}
                carry = {k: part(gl, 6 - k0 + k, nd) for k in range(gspill)}
            step(1, 1, n, fm, hooks)
            if n + 1 < NN:
                fm2 = dict(carry)
                if n + 1 >= NN - 2:
                    tl = part(tfill(2, 0), n + 1 - (NN - 2), 2)
                    g_ = gspill if n + 1 < NN else 0
                    for k in range(6):
                        fm2[k] = fm2.get(k, []) + part(tl, k, 6)
                step(0, 2, n + 1, fm2, [])
        arrive(('x', 3), ('x', 4))
        issue(len(Q))
        def chunk(m, slot):
            tf = tfill(jnp.minimum(m + 1, NM - 1), 1 - slot)
            for n in range(NN):
                tl = part(tf, n, NN)
                step(m, slot, n, {k: part(tl, k, 6) for k in range(6)})
        def body(i, carry):
            m = 2 * i + 2
            @pl.when(i == 1)
            def _():
                for m_ in range(5, NM): wait(x_copies(m_))
            chunk(m, 0)
            chunk(m + 1, 1)
            return carry
        with jax.named_scope('loop'):
            jax.lax.fori_loop(0, (NM - 2) // 2, body, 0)
        with jax.named_scope('outwait'):
          for m in range(NM):
            for n in range(NN):
                wait(o_copies(m, n))

    def fn(x, w, mean, var, g, b):
        return pl.pallas_call(
            kernel,
            in_specs=[pl.BlockSpec(memory_space=pl.ANY)] * 6,
            out_specs=pl.BlockSpec(memory_space=pl.ANY),
            out_shape=jax.ShapeDtypeStruct((B, S, C), x.dtype),
            scratch_shapes=[
                pltpu.VMEM((B, NCB, S + 2 * PAD, 128), BF),
                pltpu.VMEM((3, NCB, C, 128), BF),
                pltpu.VMEM((B, NCB, S, 128), BF),
                pltpu.VMEM((8, C), F32),
                pltpu.VMEM((C,), BF), pltpu.VMEM((C,), BF), pltpu.VMEM((C,), BF), pltpu.VMEM((C,), BF),
                pltpu.SemaphoreType.DMA((NM,)),
                pltpu.SemaphoreType.DMA((NN,)),
                pltpu.SemaphoreType.DMA((1,)),
                pltpu.SemaphoreType.DMA((1,)),
            ] + [pltpu.VMEM((4, C // 2, 128), U32) for _ in range(NN)] + [pltpu.VMEM((6, HT, C), U32) for _ in range(3)],
            compiler_params=pltpu.CompilerParams(vmem_limit_bytes=vmem * 2**20, flags=flags),
        )(x, w, mean, var, g, b)
    return fn


_fn = make()


@jax.jit
def pallas_standalone__batchnorm__prompt_kernel(x, w, mean, var, g, b):
    return _fn(x, w, mean, var, g, b)
```

```python
import functools

import jax
import jax.numpy as jnp
import jax.experimental.pallas as pl
import jax.experimental.pallas.tpu as pltpu

F32 = jnp.float32
BF16 = jnp.bfloat16
U32 = jnp.uint32

B, S, C = 2, 2048, 1024
EPS = 1e-5
LANES = 128
NCB = C // LANES
R = 512
CPB = S // R
NM = B * CPB
TT = R // 4
PAD = 16

PA, PB = 2.0 / 3.0, 1.5
CC = PA**2 + PB**2
SA = 1.0 / (2 * PA**2 * (PA**2 - PB**2) * PA**2)
SB = 1.0 / (2 * PB**2 * (PB**2 - PA**2) * PA**2)
DOT_ORDER = (0, 5, 1, 2, 3, 4)


def _unpack(u, i):
    return pltpu.unpack_elementwise(u, index=i, packed_dtype=BF16, unpacked_dtype=F32)


def _pack(lo, hi):
    return pltpu.pack_elementwise([lo, hi], packed_dtype=BF16)


def _input_transform(d0, d1, d2, d3, d4, d5):
    a1 = PA * d1
    pa = (PA**2) * d4 - d2
    qa = (PA**3) * d3 - a1
    pb = d4 - (PA**2) * d2
    qb = PB * d3 - a1
    return [d0 - CC * d2 + d4, pa + qa, pa - qa, pb + qb, pb - qb, d1 - CC * d3 + d5]


def _filter_transform(w0, w1, w2):
    o = PA * w1
    ea = w0 + (PA**2) * w2
    eb = (PA**2) * w0 + w2
    return [ea + o, ea - o, eb + o, eb - o]


def _output_transform(m):
    s12, d12 = m[1] + m[2], m[1] - m[2]
    s34, d34 = m[3] + m[4], m[3] - m[4]
    return [m[0] + SA * s12 + SB * s34,
            (SA * PA) * d12 + (SB * PB) * d34,
            (SA * PA**2) * s12 + (SB * PB**2) * s34,
            (SA * PA**3) * d12 + (SB * PB**3) * d34 + m[5]]


def _part(items, i, k):
    return items[i * len(items) // k:(i + 1) * len(items) // k]


def _kernel(x_hbm, w_hbm, mean_hbm, var_hbm, g_hbm, b_hbm, o_hbm,
            xs, ws, os_, coef, mean_v, var_v, g_v, b_v, xsem, wsem, osem, vsem, *gt):
    G, T = gt[:NCB], gt[NCB:]

    def batch_and_chunk(m):
        return divmod(m, CPB) if isinstance(m, int) else (m // CPB, m % CPB)

    def row0(c):
        return c * R if isinstance(c, int) else pl.multiple_of(c * R, R)

    def x_copies(m):
        b, c = divmod(m, CPB)
        lo = 0 if c == 0 else c * R + PAD
        hi = S if c == CPB - 1 else (c + 1) * R + PAD
        return [pltpu.make_async_copy(x_hbm.at[b, pl.ds(lo, hi - lo), pl.ds(cb * LANES, LANES)],
                                      xs.at[b, cb, pl.ds(PAD + lo, hi - lo), :], xsem.at[m])
                for cb in range(NCB)]

    def w_copies(n):
        return [pltpu.make_async_copy(w_hbm.at[k, :, pl.ds(n * LANES, LANES)], ws.at[k, n], wsem.at[n])
                for k in range(3)]

    def o_copy(m, n):
        b, c = batch_and_chunk(m)
        return pltpu.make_async_copy(os_.at[b, n, pl.ds(row0(c), R), :],
                                     o_hbm.at[b, pl.ds(row0(c), R), pl.ds(n * LANES, LANES)], osem.at[0])

    v_copies = [pltpu.make_async_copy(src, dst, vsem.at[0]) for src, dst in
                ((mean_hbm, mean_v), (var_hbm, var_v), (g_hbm, g_v), (b_hbm, b_v))]

    def copies(item):
        return x_copies(item[1]) if item[0] == "x" else w_copies(item[1])

    def sync(waits, starts):
        for item in waits:
            for cp in copies(item):
                cp.wait()
        for item in starts:
            for cp in copies(item):
                cp.start()

    def X(*idx):
        return [("x", i) for i in idx]

    def W(*idx):
        return [("w", i) for i in idx]

    for cp in v_copies:
        cp.start()
    sync([], X(0) + W(0))

    zeros = jnp.zeros((PAD, LANES), BF16)
    for b in range(B):
        for cb in range(NCB):
            xs[b, cb, 0:PAD, :] = zeros
            xs[b, cb, PAD + S:PAD + S + PAD, :] = zeros

    def g_piece(n, r):
        rows = slice(r, r + 8)
        u = [ws.at[k, n].bitcast(U32)[rows, :] for k in range(3)]
        even = _filter_transform(*[_unpack(v, 0) for v in u])
        odd = _filter_transform(*[_unpack(v, 1) for v in u])
        seen = None
        for j in range(4):
            p = _pack(even[j], odd[j])
            G[n][j, rows, :] = p
            seen = p if seen is None else seen | p
        return seen

    def t_piece(m, slot, cb, t0):
        b, c = batch_and_chunk(m)
        xu = xs.at[b, cb, pl.ds(row0(c), R + 2 * PAD), :].bitcast(U32)
        base = PAD // 2 + 2 * t0
        u = [xu[pl.ds(base + o, 8, stride=4), :] for o in range(-1, 5)]
        lo = [None] + [_unpack(v, 0) for v in u[1:]]
        hi = [_unpack(v, 1) for v in u[:5]]
        even = _input_transform(hi[0], lo[1], hi[1], lo[2], hi[2], lo[3])
        odd = _input_transform(hi[2], lo[3], hi[3], lo[4], hi[4], lo[5])
        seen = None
        for j in range(6):
            p = _pack(even[j], odd[j])
            T[slot][j, t0 // 2:t0 // 2 + 8, cb * LANES:(cb + 1) * LANES] = p
            seen = p if seen is None else seen | p
        return seen

    def g_pieces(n):
        return [functools.partial(g_piece, n, r) for r in range(0, C // 2, 8)]

    def t_pieces(m, slot):
        return [functools.partial(t_piece, m, slot, cb, t0)
                for cb in range(NCB) for t0 in range(0, TT, 16)]

    zero_bits = []

    def step(m, slot, n, pieces=None, hooks=None):
        b, c = batch_and_chunk(m)
        cols = slice(n * LANES, (n + 1) * LANES)
        prod = {}
        for k, j in enumerate(DOT_ORDER):
            if hooks and k in hooks:
                hooks[k]()
            seen = None
            for piece in (pieces or {}).get(k, ()):
                v = piece()
                seen = v if seen is None else seen | v
            t = T[slot]
            if seen is None:
                lhs = t[j]
            else:
                r, q = TT // 2 - 8, C - LANES
                last = jnp.concatenate([t[j, r:, :q], t[j, r:, q:] | (seen & zero_bits[0])], axis=1)
                lhs = jnp.concatenate([t[j, :r, :], last], axis=0)
            if j == 0:
                rhs = ws.at[0, n].bitcast(U32)[...]
            elif j == 5:
                rhs = ws.at[2, n].bitcast(U32)[...]
            else:
                rhs = G[n][j - 1]
            prod[j] = jnp.dot(pltpu.bitcast(lhs, BF16), pltpu.bitcast(rhs, BF16),
                              preferred_element_type=F32)

        def bn_silu(y):
            h = y * coef[0:1, cols] + coef[1:2, cols]
            return h * jnp.tanh(h) + h

        y = [bn_silu(v) for v in _output_transform(prod)]
        ou = os_.at[b, n, pl.ds(row0(c), R), :].bitcast(U32)
        ou[pl.ds(0, TT, stride=2), :] = _pack(y[0], y[1])
        ou[pl.ds(1, TT, stride=2), :] = _pack(y[2], y[3])
        o_copy(m, n).start()

    sync(X(0), W(1))
    for piece in t_pieces(0, 2):
        piece()
    for cp in v_copies:
        cp.wait()
    vec = lambda ref: ref[...].astype(F32).reshape(1, C)
    scale = vec(g_v) * jax.lax.rsqrt(vec(var_v) + EPS)
    coef[0:1, :] = 0.5 * scale
    coef[1:2, :] = 0.5 * (vec(b_v) - vec(mean_v) * scale)
    zero_bits.append((pltpu.bitcast(jnp.broadcast_to(scale[:, :LANES], (8, LANES)), U32) >> 16) >> 16)

    for n, waits, starts in ((0, W(0), X(1)), (1, W(1), W(2, 3))):
        sync(waits, starts)
        gp = g_pieces(n)
        step(0, 2, n, {0: _part(gp, 0, 2), 1: _part(gp, 1, 2)})
    sync(X(1), W(4, 5))
    for piece in t_pieces(1, 1):
        piece()

    order = [(1, 0), (1, 1)]
    for n in range(2, NCB):
        order += [(0, n), (1, n)]
    pieces = {st: {} for st in order}

    def spread(items, slots):
        for i, (st, k) in enumerate(slots):
            pieces[st][k] = pieces[st].get(k, []) + _part(items, i, len(slots))

    for n in range(2, NCB):
        spread(g_pieces(n), [((1, n - 1), k) for k in range(6)] + [((0, n), k) for k in range(3)])
    spread(t_pieces(2, 0), [((0, 6), k) for k in range(3, 6)] + [((0, 7), k) for k in range(3, 6)]
           + [((1, 7), k) for k in range(6)])
    arrivals = {(1, 1): (W(2), W(6, 7) + X(2)), (1, 2): (W(3), []), (1, 3): (W(4, 5), X(3, 4)),
                (1, 5): (W(6, 7) + X(2), X(5, 6, 7))}
    for st in order:
        hooks = {0: functools.partial(sync, *arrivals[st])} if st in arrivals else None
        step(st[0], 2 if st[0] == 0 else 1, st[1], pieces[st], hooks)
    sync(X(3, 4), [])

    def chunk(m, slot):
        nxt = t_pieces(jnp.minimum(m + 1, NM - 1), 1 - slot)
        for n in range(NCB):
            mine = _part(nxt, n, NCB)
            step(m, slot, n, {k: _part(mine, k, 6) for k in range(6)})

    def two_chunks(i, carry):
        @pl.when(i == 1)
        def _():
            sync(X(5, 6, 7), [])

        chunk(2 * i + 2, 0)
        chunk(2 * i + 3, 1)
        return carry

    jax.lax.fori_loop(0, (NM - 2) // 2, two_chunks, 0)
    for m in range(NM):
        for n in range(NCB):
            o_copy(m, n).wait()


@jax.jit
def pallas_standalone__batchnorm__prompt_kernel(x, w, mean, var, g, b):
    assert x.shape == (B, S, C) and w.shape == (3, C, C)
    return pl.pallas_call(
        _kernel,
        in_specs=[pl.BlockSpec(memory_space=pl.ANY)] * 6,
        out_specs=pl.BlockSpec(memory_space=pl.ANY),
        out_shape=jax.ShapeDtypeStruct((B, S, C), x.dtype),
        scratch_shapes=[
            pltpu.VMEM((B, NCB, S + 2 * PAD, LANES), BF16),
            pltpu.VMEM((3, NCB, C, LANES), BF16),
            pltpu.VMEM((B, NCB, S, LANES), BF16),
            pltpu.VMEM((8, C), F32),
            pltpu.VMEM((C,), BF16), pltpu.VMEM((C,), BF16), pltpu.VMEM((C,), BF16), pltpu.VMEM((C,), BF16),
            pltpu.SemaphoreType.DMA((NM,)),
            pltpu.SemaphoreType.DMA((NCB,)),
            pltpu.SemaphoreType.DMA((1,)),
            pltpu.SemaphoreType.DMA((1,)),
        ] + [pltpu.VMEM((4, C // 2, LANES), U32) for _ in range(NCB)]
          + [pltpu.VMEM((6, TT // 2, C), U32) for _ in range(3)],
        compiler_params=pltpu.CompilerParams(vmem_limit_bytes=100 * 2**20),
    )(x, w, mean, var, g, b)
```

```python
import functools

import jax
import jax.numpy as jnp
import jax.experimental.pallas as pl
import jax.experimental.pallas.tpu as pltpu

F32 = jnp.float32
BF16 = jnp.bfloat16
U32 = jnp.uint32

B, S, C = 2, 2048, 1024
EPS = 1e-5
LANES = 128
NCB = C // LANES
R = 512
CPB = S // R
NM = B * CPB
TT = R // 4
PAD = 16

PA, PB = 2.0 / 3.0, 1.5
CC = PA**2 + PB**2
SA = 1.0 / (2 * PA**2 * (PA**2 - PB**2) * PA**2)
SB = 1.0 / (2 * PB**2 * (PB**2 - PA**2) * PA**2)
DOT_ORDER = (0, 5, 1, 2, 3, 4)


def _unpack(u, i):
    return pltpu.unpack_elementwise(u, index=i, packed_dtype=BF16, unpacked_dtype=F32)


def _pack(lo, hi):
    return pltpu.pack_elementwise([lo, hi], packed_dtype=BF16)


def _input_transform(d0, d1, d2, d3, d4, d5):
    a1 = PA * d1
    pa = (PA**2) * d4 - d2
    qa = (PA**3) * d3 - a1
    pb = d4 - (PA**2) * d2
    qb = PB * d3 - a1
    return [d0 - CC * d2 + d4, pa + qa, pa - qa, pb + qb, pb - qb, d1 - CC * d3 + d5]


def _filter_transform(w0, w1, w2):
    o = PA * w1
    ea = w0 + (PA**2) * w2
    eb = (PA**2) * w0 + w2
    return [ea + o, ea - o, eb + o, eb - o]


def _output_transform(m):
    s12, d12 = m[1] + m[2], m[1] - m[2]
    s34, d34 = m[3] + m[4], m[3] - m[4]
    return [m[0] + SA * s12 + SB * s34,
            (SA * PA) * d12 + (SB * PB) * d34,
            (SA * PA**2) * s12 + (SB * PB**2) * s34,
            (SA * PA**3) * d12 + (SB * PB**3) * d34 + m[5]]


def _part(items, i, k):
    return items[i * len(items) // k:(i + 1) * len(items) // k]


def _kernel(x_hbm, w_hbm, mean_hbm, var_hbm, g_hbm, b_hbm, o_hbm,
            xs, ws, os_, coef, mean_v, var_v, g_v, b_v, xsem, wsem, osem, vsem, *gt):
    G, T = gt[:NCB], gt[NCB:]

    def batch_and_chunk(m):
        return divmod(m, CPB) if isinstance(m, int) else (m // CPB, m % CPB)

    def row0(c):
        return c * R if isinstance(c, int) else pl.multiple_of(c * R, R)

    def x_copies(m):
        b, c = divmod(m, CPB)
        lo = 0 if c == 0 else c * R + PAD
        hi = S if c == CPB - 1 else (c + 1) * R + PAD
        return [pltpu.make_async_copy(x_hbm.at[b, pl.ds(lo, hi - lo), pl.ds(cb * LANES, LANES)],
                                      xs.at[b, cb, pl.ds(PAD + lo, hi - lo), :], xsem.at[m])
                for cb in range(NCB)]

    def w_copies(n):
        return [pltpu.make_async_copy(w_hbm.at[k, :, pl.ds(n * LANES, LANES)], ws.at[k, n], wsem.at[n])
                for k in range(3)]

    def o_copy(m, n):
        b, c = batch_and_chunk(m)
        return pltpu.make_async_copy(os_.at[b, n, pl.ds(row0(c), R), :],
                                     o_hbm.at[b, pl.ds(row0(c), R), pl.ds(n * LANES, LANES)], osem.at[0])

    v_copies = [pltpu.make_async_copy(src, dst, vsem.at[0]) for src, dst in
                ((mean_hbm, mean_v), (var_hbm, var_v), (g_hbm, g_v), (b_hbm, b_v))]

    def copies(item):
        return x_copies(item[1]) if item[0] == "x" else w_copies(item[1])

    def sync(waits, starts):
        for item in waits:
            for cp in copies(item):
                cp.wait()
        for item in starts:
            for cp in copies(item):
                cp.start()

    def X(*idx):
        return [("x", i) for i in idx]

    def W(*idx):
        return [("w", i) for i in idx]

    for cp in v_copies:
        cp.start()
    sync([], X(0) + W(0))

    zeros = jnp.zeros((PAD, LANES), BF16)
    for b in range(B):
        for cb in range(NCB):
            xs[b, cb, 0:PAD, :] = zeros
            xs[b, cb, PAD + S:PAD + S + PAD, :] = zeros

    def g_piece(n, r):
        rows = slice(r, r + 8)
        u = [ws.at[k, n].bitcast(U32)[rows, :] for k in range(3)]
        even = _filter_transform(*[_unpack(v, 0) for v in u])
        odd = _filter_transform(*[_unpack(v, 1) for v in u])
        seen = None
        for j in range(4):
            p = _pack(even[j], odd[j])
            G[n][j, rows, :] = p
            seen = p if seen is None else seen | p
        return seen

    def t_piece(m, slot, cb, t0):
        b, c = batch_and_chunk(m)
        xu = xs.at[b, cb, pl.ds(row0(c), R + 2 * PAD), :].bitcast(U32)
        base = PAD // 2 + 2 * t0
        u = [xu[pl.ds(base + o, 8, stride=4), :] for o in range(-1, 5)]
        lo = [None] + [_unpack(v, 0) for v in u[1:]]
        hi = [_unpack(v, 1) for v in u[:5]]
        even = _input_transform(hi[0], lo[1], hi[1], lo[2], hi[2], lo[3])
        odd = _input_transform(hi[2], lo[3], hi[3], lo[4], hi[4], lo[5])
        seen = None
        for j in range(6):
            p = _pack(even[j], odd[j])
            T[slot][j, t0 // 2:t0 // 2 + 8, cb * LANES:(cb + 1) * LANES] = p
            seen = p if seen is None else seen | p
        return seen

    def g_pieces(n):
        return [functools.partial(g_piece, n, r) for r in range(0, C // 2, 8)]

    def t_pieces(m, slot):
        return [functools.partial(t_piece, m, slot, cb, t0)
                for cb in range(NCB) for t0 in range(0, TT, 16)]

    zero_bits = []

    def step(m, slot, n, pieces=None, hooks=None, send=True):
        b, c = batch_and_chunk(m)
        cols = slice(n * LANES, (n + 1) * LANES)
        prod = {}
        for k, j in enumerate(DOT_ORDER):
            if hooks and k in hooks:
                hooks[k]()
            seen = None
            for piece in (pieces or {}).get(k, ()):
                v = piece()
                seen = v if seen is None else seen | v
            t = T[slot]
            if seen is None:
                lhs = t[j]
            else:
                r, q = TT // 2 - 8, C - LANES
                last = jnp.concatenate([t[j, r:, :q], t[j, r:, q:] | (seen & zero_bits[0])], axis=1)
                lhs = jnp.concatenate([t[j, :r, :], last], axis=0)
            if j == 0:
                rhs = ws.at[0, n].bitcast(U32)[...]
            elif j == 5:
                rhs = ws.at[2, n].bitcast(U32)[...]
            else:
                rhs = G[n][j - 1]
            prod[j] = jnp.dot(pltpu.bitcast(lhs, BF16), pltpu.bitcast(rhs, BF16),
                              preferred_element_type=F32)

        def bn_silu(y):
            h = y * coef[0:1, cols] + coef[1:2, cols]
            return h * jnp.tanh(h) + h

        y = [bn_silu(v) for v in _output_transform(prod)]
        ou = os_.at[b, n, pl.ds(row0(c), R), :].bitcast(U32)
        ou[pl.ds(0, TT, stride=2), :] = _pack(y[0], y[1])
        ou[pl.ds(1, TT, stride=2), :] = _pack(y[2], y[3])
        if send:
            o_copy(m, n).start()

    sync(X(0), W(1))
    for piece in t_pieces(0, 2):
        piece()
    for cp in v_copies:
        cp.wait()
    vec = lambda ref: ref[...].astype(F32).reshape(1, C)
    scale = vec(g_v) * jax.lax.rsqrt(vec(var_v) + EPS)
    coef[0:1, :] = 0.5 * scale
    coef[1:2, :] = 0.5 * (vec(b_v) - vec(mean_v) * scale)
    zero_bits.append((pltpu.bitcast(jnp.broadcast_to(scale[:, :LANES], (8, LANES)), U32) >> 16) >> 16)

    for n, waits, starts in ((0, W(0), X(1)), (1, W(1), W(2, 3))):
        sync(waits, starts)
        gp = g_pieces(n)
        step(0, 2, n, {0: _part(gp, 0, 2), 1: _part(gp, 1, 2)}, send=False)
    sync(X(1), W(4, 5))
    for piece in t_pieces(1, 1):
        piece()

    order = [(1, 0), (1, 1)]
    for n in range(2, NCB):
        order += [(0, n), (1, n)]
    pieces = {st: {} for st in order}

    def spread(items, slots):
        for i, (st, k) in enumerate(slots):
            pieces[st][k] = pieces[st].get(k, []) + _part(items, i, len(slots))

    for n in range(2, NCB):
        first = 4 if n == 5 else 0
        spread(g_pieces(n), [((1, n - 1), k) for k in range(first, 6)] + [((0, n), k) for k in range(3)])
    spread(t_pieces(2, 0), [((0, n), k) for n in (5, 6, 7) for k in range(3, 6)]
           + [((1, 7), k) for k in range(6)])
    arrivals = {(1, 1): (0, W(2), W(6, 7) + X(2)),
                (1, 2): (0, W(3, 4), []),
                (1, 4): (4, W(5, 6, 7) + X(2), X(3, 4))}
    for st in order:
        if st == (0, 5):
            for m, n in [(m, n) for n in range(5) for m in range(2)]:
                o_copy(m, n).start()
        hooks = None
        if st in arrivals:
            k, waits, starts = arrivals[st]
            hooks = {k: functools.partial(sync, waits, starts)}
        step(st[0], 2 if st[0] == 0 else 1, st[1], pieces[st], hooks, send=st[1] >= 5)
    sync(X(3, 4), X(5, 6, 7))

    def chunk(m, slot):
        nxt = t_pieces(jnp.minimum(m + 1, NM - 1), 1 - slot)
        for n in range(NCB):
            mine = _part(nxt, n, NCB)
            step(m, slot, n, {k: _part(mine, k, 6) for k in range(6)})

    def two_chunks(i, carry):
        @pl.when(i == 1)
        def _():
            sync(X(5, 6, 7), [])

        chunk(2 * i + 2, 0)
        chunk(2 * i + 3, 1)
        return carry

    jax.lax.fori_loop(0, (NM - 2) // 2, two_chunks, 0)
    for m in range(NM):
        for n in range(NCB):
            o_copy(m, n).wait()


@jax.jit
def pallas_standalone__batchnorm__prompt_kernel(x, w, mean, var, g, b):
    assert x.shape == (B, S, C) and w.shape == (3, C, C)
    return pl.pallas_call(
        _kernel,
        in_specs=[pl.BlockSpec(memory_space=pl.ANY)] * 6,
        out_specs=pl.BlockSpec(memory_space=pl.ANY),
        out_shape=jax.ShapeDtypeStruct((B, S, C), x.dtype),
        scratch_shapes=[
            pltpu.VMEM((B, NCB, S + 2 * PAD, LANES), BF16),
            pltpu.VMEM((3, NCB, C, LANES), BF16),
            pltpu.VMEM((B, NCB, S, LANES), BF16),
            pltpu.VMEM((8, C), F32),
            pltpu.VMEM((C,), BF16), pltpu.VMEM((C,), BF16), pltpu.VMEM((C,), BF16), pltpu.VMEM((C,), BF16),
            pltpu.SemaphoreType.DMA((NM,)),
            pltpu.SemaphoreType.DMA((NCB,)),
            pltpu.SemaphoreType.DMA((1,)),
            pltpu.SemaphoreType.DMA((1,)),
        ] + [pltpu.VMEM((4, C // 2, LANES), U32) for _ in range(NCB)]
          + [pltpu.VMEM((6, TT // 2, C), U32) for _ in range(3)],
        compiler_params=pltpu.CompilerParams(vmem_limit_bytes=64 * 2**20),
    )(x, w, mean, var, g, b)
```
